```python
import os as _os
_os.environ.setdefault("JAX_PLATFORMS", "cpu")
import jax
import jax.numpy as jnp

def _softmax(x, axis=-1):
    return jax.nn.softmax(x, axis=axis)
def _gelu(x):
    return jax.nn.gelu(x, approximate=True)
def _silu(x):
    return jax.nn.silu(x)
def _sigmoid(x):
    return jax.nn.sigmoid(x)
def _layernorm(x, axis=-1, eps=1e-5):
    m = jnp.mean(x, axis=axis, keepdims=True)
    v = jnp.var(x, axis=axis, keepdims=True)
    return (x - m) / jnp.sqrt(v + eps)
def _scatter_add(tgt, idx, src, axis=0):
    return tgt.at[idx].add(src)
def _segment_sum(src, seg, n):
    return jax.ops.segment_sum(src, seg, n)
class _Rng:
    def __init__(self, key):
        self._k = key
    def _next(self):
        self._k, sub = jax.random.split(self._k)
        return sub
    def normal(self, shape):
        return jax.random.normal(self._next(), shape, dtype=jnp.bfloat16)
    def randint(self, lo, hi, shape):
        return jax.random.randint(self._next(), shape, lo, hi, dtype=jnp.int32)
    def uniform(self, shape, lo=0.0, hi=1.0):
        return jax.random.uniform(self._next(), shape, jnp.bfloat16, lo, hi)
    def permutation(self, n):
        return jax.random.permutation(self._next(), n)


kernel_name = 'standalone__glu_gated_bilinear__prompt'

def setup_inputs():
    _rng = _Rng(jax.random.key(int.from_bytes(__import__("os").urandom(4), "little")))
    _w = (lambda a: (lambda t: t.astype(jnp.bfloat16) if jnp.issubdtype(t.dtype, jnp.floating) else t)(jnp.asarray(a)))
    B, S, D, F = 1, 2048, 640, 1728
    return {
        "x": _w((lambda *s: _rng.normal(s) * 0.05)(B, S, D)),
        "w_gate": _w((lambda *s: _rng.normal(s) * 0.05)(D, F) * (D ** -0.5)),
        "w_up": _w((lambda *s: _rng.normal(s) * 0.05)(D, F) * (D ** -0.5)),
        "w_down": _w((lambda *s: _rng.normal(s) * 0.05)(F, D) * (F ** -0.5)),
    }

def reference(x, w_gate, w_up, w_down):
    g = jnp.einsum("bsd,df->bsf", x, w_gate)
    u = jnp.einsum("bsd,df->bsf", x, w_up)
    h = g * u
    return jnp.einsum("bsf,fd->bsd", h, w_down)
```

```python
import jax
import jax.numpy as jnp
from jax import lax
import jax.experimental.pallas as pl
import jax.experimental.pallas.tpu as pltpu

T = 128
B = 128
_NT = (((1,), (1,)), ((), ()))
_NN = (((1,), (0,)), ((), ()))


def _products(rows, cols, diag):
    kind = {(k, n): t for k, n, t in diag}
    paired, pairs = set(), []
    for k, n, t in diag:
        for k2, n2, t2 in diag:
            if (t, t2) != (1, 2) or k == k2 or n == n2:
                continue
            if any(c in kind or c in paired for c in ((k, n2), (k2, n))):
                continue
            paired.update(((k, n2), (k2, n)))
            pairs.append((k, n, k2, n2))
    prods = []
    for k, n, t in diag:
        both = ((1, 0, k), (1, 1, k))
        if t == 1:
            part = [(c, d) for a, b, c, d in pairs if (a, b) == (k, n)]
        else:
            part = [(a, b) for a, b, c, d in pairs if (c, d) == (k, n)]
        col = ((1, k, n),) + tuple((1, a, n) for a, _ in part)
        row = ((1, k, n),) + tuple((-1, k, b) for _, b in part)
        if t == 1:
            prods.append((((1, 0, k),), col, ((1, 0, n), (-1, 1, n))))
            prods.append((both, row, ((1, 1, n),)))
        else:
            prods.append((both, row, ((1, 0, n),)))
            prods.append((((1, 1, k),), col, ((1, 1, n), (-1, 0, n))))
    for k, n, k2, n2 in pairs:
        s = 1 if k2 > k else -1
        hi, lo = max(k, k2), min(k, k2)
        prods.append((((1, 0, k), (1, 1, k2)), ((1, k, n2), (1, k2, n)), ((1, 0, n2), (1, 1, n))))
        prods.append((((1, 0, hi), (-1, 0, lo)), ((1, k2, n),), ((s, 0, n2), (s, 0, n))))
        prods.append((((1, 1, hi), (-1, 1, lo)), ((1, k, n2),), ((-s, 1, n2), (-s, 1, n))))
    for k in rows:
        for n in cols:
            if (k, n) not in kind and (k, n) not in paired:
                for h in (0, 1):
                    prods.append((((1, h, k),), ((1, k, n),), ((1, h, n),)))
    return prods


def _in_quads(prods):
    left, out = list(prods), []
    while left:
        seen = set()
        for _ in range(min(4, len(left))):
            cost = [len({d[1:] for d in p[2]} - seen) for p in left]
            p = left.pop(cost.index(min(cost)) if seen else 0)
            seen.update(d[1:] for d in p[2])
            out.append(p)
    return out


def _signed_sum(terms, get):
    acc = None
    for sign, *idx in sorted(terms, key=lambda t: -t[0]):
        v = get(*idx)
        acc = v if acc is None else (acc + v if sign > 0 else acc - v)
    return acc


@jax.jit
def pallas_standalone__glu_gated_bilinear__prompt_kernel(
    x: jax.Array,
    w_gate: jax.Array,
    w_up: jax.Array,
    w_down: jax.Array,
):
    batch, seq, D = x.shape
    S = batch * seq
    F = w_gate.shape[1]
    assert (S, D, F) == (2048, 640, 1728)
    f32, bf16 = jnp.float32, x.dtype
    niter = 2
    R = S // 2 // niter
    blocks = tuple(range(R // B))

    kt = range(D // T)
    stage1 = []
    for base in (0, 5):
        cols = [(t, base + f) for t in "gu" for f in range(5)]
        diag = [(f, ("g", base + f), 1) for f in range(5)] + [(f, ("u", base + f), 2) for f in range(5)]
        stage1.append(_products(kt, cols, diag))
    cols = [("g", 10), ("u", 10), ("g", 11), ("u", 11), ("g", 12), ("u", 12), ("m", 13)]
    diag = [(0, 1, 2), (0, 5, 2), (1, 5, 2), (1, 6, 1), (2, 2, 1), (2, 4, 2), (3, 0, 1), (3, 2, 2), (4, 3, 1), (4, 6, 2)]
    stage1.append(_products(kt, cols, [(k, cols[n], t) for k, n, t in diag]))
    stage2 = _products(range(10), kt, [(n, n, 1) for n in kt] + [(5 + n, n, 2) for n in kt])
    stage2r = _products(range(10, 14), kt, [(10, 0, 1), (11, 1, 1), (12, 2, 2), (13, 3, 2), (11, 4, 2), (13, 4, 1)])

    X = lambda h, b0, b1: (("x", h, b0, b1), "x", h * R + b0 * B, (b1 - b0) * B)
    W = lambda a, f: ((a, f), a, f * T, T)
    plan = [X(0, 0, 2), W("g", 0), W("g", 1), X(0, 2, 4), W("g", 2), W("g", 3), W("g", 4), X(1, 0, 4)]
    plan += [W("u", f) for f in range(5)]
    plan += [W(a, f) for f in range(5, 10) for a in "gu"]
    plan += [((a, 10), a, 10 * T, F - 10 * T) for a in "gu"]
    plan += [(("d", 0), "d", 0, 10 * T), (("d", 10), "d", 10 * T, F - 10 * T)]
    rank = {p[0]: i for i, p in enumerate(plan)}

    def w_keys(n):
        t, f = n
        return [("g", 10), ("u", 10)] if t == "m" else [(t, min(f, 10))]

    def x_key(h, b):
        return next(k for k in rank if k[0] == "x" and k[1] == h and k[2] <= b < k[3])

    def arrival(prod, b):
        lhs, rhs, _ = prod
        return max([rank[x_key(h, b)] for _, h, _ in lhs] + [rank[c] for _, _, n in rhs for c in w_keys(n)])

    early = [p for p in stage1[0] if all(h == 0 for _, h, _ in p[0])]
    late = sorted((p for p in stage1[0] if p not in early), key=lambda p: arrival(p, 0))
    pieces = {}
    for p in early:
        for b in blocks:
            pieces.setdefault((arrival(p, b), p), []).append(b)
    order = sorted(pieces, key=lambda c: (c[0], arrival(c[1], 0), len(c[1][1])))
    sched = [(1, p, tuple(pieces[a, p])) for a, p in order]
    sched += [(1, p, blocks) for p in late + _in_quads(stage1[1]) + _in_quads(stage1[2])]
    single = sorted((p for p in stage2 if len(p[2]) == 1), key=lambda p: (p[2][0][2], p[2][0][1]))
    middle = _in_quads([p for p in stage2 + stage2r if p not in single])
    sched += [(2, p, blocks) for p in single[:2] + middle + single[2:]]

    def kernel(x_hbm, wg_hbm, wu_hbm, wd_hbm, o_hbm, xv, gv, uv, dv, ov, in_sem, out_sem):
        hbm = dict(x=x_hbm, g=wg_hbm, u=wu_hbm, d=wd_hbm)
        vmem = dict(x=xv, g=gv, u=uv, d=dv)

        def copy(it, i):
            _, a, r0, nr = plan[i]
            src = hbm[a].at[pl.ds(it * 2 * R + r0 if a == "x" else r0, nr)]
            return pltpu.make_async_copy(src, vmem[a].at[it, pl.ds(r0, nr)], in_sem.at[it * len(plan) + i])

        for it in range(niter):
            for i in range(len(plan)):
                copy(it, i).start()

        def body(it, carry):
            pending = set(rank)

            def need(key):
                if key in pending:
                    copy(it, rank[key]).wait()
                    pending.discard(key)

            xr, gr, ur, dr = xv.at[it], gv.at[it], uv.at[it], dv.at[it]

            def w1(k, n):
                t, f = n
                for c in w_keys(n):
                    need(c)
                if t == "m":
                    return jnp.concatenate([gr[f * T:F, k * T:(k + 1) * T], ur[f * T:F, k * T:(k + 1) * T]], axis=0)
                return (gr if t == "g" else ur)[f * T:(f + 1) * T, k * T:(k + 1) * T]

            def w2(k, n):
                need(("d", 0 if k < 10 else 10))
                if (k + 1) * T > F:
                    pad = jnp.zeros(((k + 1) * T - F, T), bf16)
                    return jnp.concatenate([dr[k * T:F, n * T:(n + 1) * T], pad], axis=0)
                return dr[k * T:(k + 1) * T, n * T:(n + 1) * T]

            def weight(stage, rhs):
                get = w1 if stage == 1 else w2
                if len(rhs) == 1:
                    return get(*rhs[0][1:])
                return _signed_sum(rhs, lambda k, n: get(k, n).astype(f32)).astype(bf16)

            def x_block(h, k, b):
                need(x_key(h, b))
                return xr[h * R + b * B:h * R + (b + 1) * B, k * T:(k + 1) * T]

            x_sums = {}

            def x_operand(lhs, b):
                if len(lhs) == 1:
                    return x_block(*lhs[0][1:], b)
                if (lhs, b) not in x_sums:
                    x_sums[lhs, b] = _signed_sum(lhs, lambda h, k: x_block(h, k, b).astype(f32)).astype(bf16)
                return x_sums[lhs, b]

            acc, left, hid = {}, {}, {}
            for _, (_, _, dst), bs in sched:
                for _, h, n in dst:
                    for b in bs:
                        left[h, n, b] = left.get((h, n, b), 0) + 1

            for stage, (lhs, rhs, dst), bs in sched:
                if stage == 1:
                    a = [x_operand(lhs, b) for b in bs]
                else:
                    a = [_signed_sum(lhs, lambda h, k: hid[h, k, b]).astype(bf16) for b in bs]
                r = lax.dot_general(jnp.concatenate(a, axis=0), weight(stage, rhs),
                                    _NT if stage == 1 else _NN, preferred_element_type=f32)
                for s, h, n in dst:
                    for j, b in enumerate(bs):
                        key, rb = (h, n, b), r[j * B:(j + 1) * B]
                        if key not in acc:
                            acc[key] = (s, rb)
                        else:
                            s0, v = acc[key]
                            if s0 > 0:
                                acc[key] = (1, v + rb if s > 0 else v - rb)
                            else:
                                acc[key] = (1, rb - v) if s > 0 else (-1, v + rb)
                        left[key] -= 1
                        if left[key]:
                            continue
                        sign, v = acc[key]
                        assert sign > 0
                        if stage == 2:
                            rows = pl.ds(it * 2 * R + h * R + b * B, B)
                            ov[rows, n * T:(n + 1) * T] = v.astype(ov.dtype)
                            blk = (rows, pl.ds(n * T, T))
                            pltpu.make_async_copy(ov.at[blk], o_hbm.at[blk], out_sem).start()
                        elif n[0] == "m":
                            hid[h, n[1], b] = v * pltpu.roll(v, T // 2, 1)
                        else:
                            other = (h, ("u" if n[0] == "g" else "g", n[1]), b)
                            if left[other] == 0:
                                hid[h, n[1], b] = v * acc[other][1]
            assert not pending
            return carry

        lax.fori_loop(0, niter, body, 0)
        pltpu.make_async_copy(ov, o_hbm, out_sem).wait()

    args = (x.reshape(S, D), w_gate.T, w_up.T, w_down)
    args = tuple(pltpu.with_memory_space_constraint(a, pltpu.HBM) for a in args)
    out = pl.pallas_call(
        kernel,
        in_specs=[pl.BlockSpec(memory_space=pltpu.HBM)] * 4,
        out_specs=pl.BlockSpec(memory_space=pltpu.HBM),
        out_shape=jax.ShapeDtypeStruct((S, D), x.dtype),
        scratch_shapes=[
            pltpu.VMEM((niter, 2 * R, D), x.dtype),
            pltpu.VMEM((niter, F, D), x.dtype),
            pltpu.VMEM((niter, F, D), x.dtype),
            pltpu.VMEM((niter, F, D), x.dtype),
            pltpu.VMEM((S, D), x.dtype),
            pltpu.SemaphoreType.DMA((niter * len(plan),)),
            pltpu.SemaphoreType.DMA(()),
        ],
        compiler_params=pltpu.CompilerParams(
            vmem_limit_bytes=100 * 1024 * 1024,
            flags={"XLA_TPU_RESCHEDULE_DMA_DONES": True},
            disable_semaphore_checks=True,
        ),
    )(*args)
    return out.reshape(batch, seq, D)
```

```python
import jax
import jax.numpy as jnp
from jax import lax
import jax.experimental.pallas as pl
import jax.experimental.pallas.tpu as pltpu

T = 128
HALF = T // 2
ROWS = 512
BLOCK = 128

_ALPHA = {1: (1, 0), 2: (0, 1), 3: (-1, -1)}
_BETA = {1: (0, -1), 2: (1, 0), 3: (-1, 1)}


def _combine(*terms):
    out = {}
    for scale, vec in terms:
        for key, value in vec.items():
            out[key] = out.get(key, 0) + scale * value
    return {key: value for key, value in out.items() if value}


def _hopcroft_kerr(n_rows, n_cols, seeds, pairs):
    products, index, cell = [], [], {}

    def form(table, t, vec):
        return {(h, i): c * v for h, c in enumerate(table[t]) if c for i, v in vec.items()}

    def product(u, v):
        products.append((u, v))
        return {len(products) - 1: 1}

    def orientation(i, j):
        return 1 if (j - i) % 3 == 1 else -1

    for k, n, t in seeds:
        a, y = {k: 1}, {n: 1}
        i, j = [d for d in (1, 2, 3) if d != t]
        own = {(i, j): product(form(_ALPHA, i, a), form(_BETA, j, y)),
               (j, i): product(form(_ALPHA, j, a), form(_BETA, i, y))}
        index.append((a, y, t, own))
        cell[k, n] = _combine((orientation(i, j), own[i, j]), (orientation(j, i), own[j, i]))
    for first, second, sign_a, sign_y in pairs:
        a1, y1, s, own1 = index[first]
        a2, y2, t, own2 = index[second]
        a1, y1 = _combine((sign_a, a1)), _combine((sign_y, y1))
        own1 = {d: _combine((sign_a * sign_y, e)) for d, e in own1.items()}
        u = 6 - s - t
        a, y = _combine((1, a2), (-1, a1)), _combine((1, y1), (1, y2))
        p1 = product(_combine((1, form(_ALPHA, t, a1)), (1, form(_ALPHA, s, a2))),
                     _combine((1, form(_BETA, s, y2)), (-1, form(_BETA, t, y1))))
        p2 = product(form(_ALPHA, t, a), form(_BETA, s, y))
        p3 = product(form(_ALPHA, s, a), form(_BETA, t, y))
        index.append((a, y, u, {(t, s): p2, (s, t): p3}))
        c = orientation(t, s)
        for av, yv, cross in (
            (a1, y2, _combine((c, p1), (c, own2[s, u]), (-c, own1[u, t]), (c, p3))),
            (a2, y1, _combine((c, p1), (c, own2[u, s]), (-c, own1[t, u]), (c, p2))),
        ):
            ((new, coef),) = [((k, n), av[k] * yv[n]) for k in av for n in yv if (k, n) not in cell]
            known = [(-coef * av[k] * yv[n], cell[k, n]) for k in av for n in yv if (k, n) != new]
            cell[new] = _combine((coef, cross), *known)

    weights = [{} for _ in products]
    for tile, expression in cell.items():
        for r, coef in expression.items():
            weights[r][tile] = coef
    total = {}
    for (u, v), w in zip(products, weights):
        for a, ca in u.items():
            for tile, cw in w.items():
                for o, co in v.items():
                    total[a, tile, o] = total.get((a, tile, o), 0) + ca * cw * co
    assert _combine((1, total)) == {
        ((h, k), (k, n), (h, n)): 1 for h in (0, 1) for k in range(n_rows) for n in range(n_cols)
    }, "the products must sum to exactly the matrix product"
    return [(u, w, v) for (u, v), w in zip(products, weights)]


def _label(products, rows, cols, transpose=False):
    out = []
    for u, w, v in products:
        if transpose:
            u, v, w = v, u, {(n, k): c for (k, n), c in w.items()}
        lhs = [(c, h, rows[k]) for (h, k), c in sorted(u.items())]
        rhs = [(c, rows[k], cols[n]) for (k, n), c in sorted(w.items())]
        dst = [(c, h, cols[n]) for (h, n), c in sorted(v.items())]
        assert all(abs(term[0]) == 1 for term in lhs + rhs + dst)
        sl, sr = lhs[0][0], max(term[0] for term in rhs)
        out.append((tuple((c * sl, h, k) for c, h, k in lhs),
                    tuple((c * sr, k, n) for c, k, n in rhs),
                    tuple((c * sl * sr, h, n) for c, h, n in dst)))
    return out


def _all_products():
    grid_5x10 = _hopcroft_kerr(
        5, 10, [(k, k, 2) for k in range(5)] + [(k, 5 + k, 1) for k in range(5)],
        [(k, 5 + j, 1, 1) for k in range(5) for j in range(5) if j != k])
    grid_5x7 = _hopcroft_kerr(
        5, 7, [(0, 0, 1), (0, 1, 2), (1, 2, 1), (1, 3, 2), (2, 4, 3), (3, 5, 2), (4, 6, 1)],
        [(0, 3, 1, 1), (1, 2, 1, -1), (4, 0, 1, -1), (5, 0, 1, 1), (6, 1, 1, 1), (4, 3, 1, -1),
         (5, 2, 1, -1), (6, 3, 1, 1), (4, 5, 1, 1), (4, 6, 1, 1), (5, 6, 1, -1), (9, 11, 1, 1),
         (12, 13, 1, -1), (18, 19, 1, 1)])
    grid_5x12 = _hopcroft_kerr(
        5, 12, [(0, 0, 1), (0, 1, 2), (0, 2, 3), (1, 3, 1), (1, 4, 2), (1, 5, 3), (2, 6, 1),
                (2, 7, 2), (3, 8, 1), (3, 9, 2), (4, 10, 1), (4, 11, 2)],
        [(0, 5, -1, -1), (1, 3, 1, -1), (2, 4, 1, 1), (6, 1, 1, 1), (7, 0, 1, -1), (8, 2, 1, 1),
         (9, 0, -1, 1), (10, 1, 1, 1), (11, 0, 1, -1), (6, 4, -1, -1), (7, 3, 1, 1), (8, 4, 1, 1),
         (9, 3, 1, -1), (10, 4, 1, -1), (11, 5, 1, -1), (6, 9, 1, 1), (7, 8, -1, -1),
         (6, 11, 1, 1), (7, 10, 1, -1), (8, 11, 1, 1), (9, 10, -1, -1), (17, 26, -1, 1),
         (15, 17, 1, 1), (22, 26, 1, 1)])
    stage1 = []
    for base in (0, 5):
        stage1 += _label(grid_5x10, range(5), [(t, base + f) for t in "gu" for f in range(5)])
    stage1 += _label(grid_5x7, range(5),
                     [("u", 10), ("g", 10), ("u", 11), ("g", 11), ("m", 13), ("g", 12), ("u", 12)])
    stage2 = _label(grid_5x12, range(12), range(5), transpose=True)
    for n in range(5):
        stage2 += [(((1, 0, "T"),), ((1, "T", n),), ((1, 0, n),)),
                   (((1, 0, "B"),), ((1, "B", n),), ((1, 1, n),)),
                   (((1, 0, "D"),), ((1, "D", n),), ((1, 0, n), (-1, 1, n)))]
    return [(1, *p) for p in stage1] + [(2, *p) for p in stage2]


_COPIES = (
    ("x", (0, 1), (0, 2), 0), ("g", (0, 1), (1, 2), 0), ("g", (1, 2), (0, 1), 0),
    ("g", (5, 6), (1, 2), 0), ("g", (6, 7), (0, 1), 0), ("x", (1, 2), (0, 2), 2),
    ("e", (10, 11), (1, 2), 3), ("e", (11, 12), (0, 1), 3), ("x", (2, 3), (0, 2), 4),
    ("x", (3, 4), (0, 2), 5), ("x", (0, 2), (2, 3), 6), ("g", (0, 2), (2, 3), 8),
    ("x", (2, 4), (2, 3), 10), ("g", (5, 7), (2, 3), 10), ("g", (2, 3), (0, 2), 12),
    ("g", (7, 8), (0, 2), 13), ("x", (0, 2), (3, 4), 14), ("g", (0, 3), (3, 4), 16),
    ("x", (2, 4), (3, 4), 17), ("g", (5, 8), (3, 4), 19), ("g", (3, 4), (0, 4), 21),
    ("g", (8, 9), (0, 4), 23), ("x", (0, 4), (4, 5), 26), ("g", (0, 4), (4, 5), 27),
    ("g", (5, 9), (4, 5), 27), ("g", (4, 5), (0, 5), 28), ("g", (9, 10), (0, 5), 29),
    ("g", (0, 1), (0, 1), 29), ("g", (5, 6), (0, 1), 29), ("g", (1, 2), (1, 2), 29),
    ("g", (6, 7), (1, 2), 30), ("g", (2, 3), (2, 3), 30), ("g", (7, 8), (2, 3), 30),
    ("x", (4, 8), (0, 2), 32), ("u", (0, 2), (0, 2), 32), ("x", (4, 8), (2, 5), 34),
    ("u", (0, 2), (2, 5), 36), ("u", (2, 5), (0, 5), 37), ("u", (5, 14), (0, 5), 43),
    ("g", (10, 14), (0, 5), 46), ("d", (0, 14), (0, 5), 55),
)

_ALL = tuple(range(ROWS // BLOCK))
_STEPS = (
    ((21, 33, 101, 113), (0,), 0), ((21, 33, 101, 113), (1,), 0), ((176, 178), (0, 1), 0),
    ((21, 33, 101, 113), (2,), 0), ((21, 33, 101, 113), (3,), 1), ((176, 178), (2, 3), 1),
    ((24, 36), (0, 1), 1), ((24, 36), (2, 3), 1), ((104,), _ALL, 0), ((116,), _ALL, 0),
    ((45,), _ALL, 0), ((48,), _ALL, 0), ((125,), _ALL, 1), ((128,), _ALL, 1),
    ((27, 39), (0, 1), 1), ((27, 39), (2, 3), 1), ((51,), _ALL, 1), ((107,), _ALL, 0),
    ((119,), _ALL, 0), ((131,), _ALL, 0), ((57,), _ALL, 0), ((60,), _ALL, 0), ((63,), _ALL, 0),
    ((137,), _ALL, 0), ((140,), _ALL, 0), ((143,), _ALL, 1), ((30, 42, 54, 66), _ALL, 0),
    ((110, 122, 134, 146), _ALL, 0), ((69, 72, 75, 78), _ALL, 0), ((149, 152, 155, 158), _ALL, 1),
    ((8,), _ALL, 1), ((32, 0, 4, 82), _ALL, 1), ((84, 80, 2, 88), _ALL, 1),
    ((34, 22, 6, 86), _ALL, 1), ((44, 10, 11, 46), _ALL, 0), ((71, 56, 59, 68), _ALL, 0),
    ((13, 12, 49, 47), _ALL, 0), ((41, 18, 3, 43), _ALL, 0), ((14, 74, 15, 76), _ALL, 0),
    ((37, 58, 79, 55), _ALL, 1), ((1, 16, 28, 26), _ALL, 0), ((17, 50, 38, 5), _ALL, 0),
    ((25, 20, 19, 29), _ALL, 0), ((196, 138, 208, 151), _ALL, 1), ((187, 73, 153, 212), _ALL, 1),
    ((185, 117, 111, 193), _ALL, 1), ((207, 139, 87, 93), _ALL, 1),
    ((182, 160, 180, 181), _ALL, 0), ((115, 129, 179, 202), _ALL, 1),
    ((126, 85, 124, 90), _ALL, 0), ((166, 189, 167, 191), _ALL, 0), ((132, 97, 130, 96), _ALL, 0),
    ((203, 173, 201, 172), _ALL, 0), ((83, 89, 157, 118), _ALL, 0), ((23, 210, 67, 147), _ALL, 1),
    ((162, 177, 163, 165), _ALL, 0), ((192, 190, 164, 194), _ALL, 1), ((77, 70, 31, 9), _ALL, 0),
    ((121, 148, 105, 40), _ALL, 1), ((170, 169, 199, 198), _ALL, 0), ((144, 142, 95, 94), _ALL, 0),
    ((81, 106, 109, 99), _ALL, 0), ((209, 53, 145, 127), _ALL, 1), ((195, 186, 214, 175), _ALL, 1),
    ((150, 141, 213, 123), _ALL, 1), ((211, 161, 174, 183), _ALL, 0),
    ((154, 103, 108, 159), _ALL, 0), ((188, 184, 215, 197), _ALL, 0),
    ((91, 120, 136, 112), _ALL, 0), ((35, 7, 62, 61), _ALL, 0), ((92, 114, 102, 100), _ALL, 0),
    ((135, 133, 98, 156), _ALL, 0), ((52, 65, 283, 64), _ALL, 1), ((171, 206, 204, 308), _ALL, 1),
    ((168, 306, 200, 205), _ALL, 1), ((260, 298, 302, 262), _ALL, 0),
    ((287, 311, 321, 289), _ALL, 1), ((305, 276, 234, 316), _ALL, 1),
    ((324, 310, 295, 293), _ALL, 0), ((238, 326, 239, 237), _ALL, 0),
    ((291, 265, 263, 249), _ALL, 0), ((320, 303, 231, 229), _ALL, 1),
    ((228, 319, 267, 224), _ALL, 0), ((266, 280, 245, 284), _ALL, 0),
    ((261, 325, 218, 304), _ALL, 1), ((250, 252, 288, 254), _ALL, 0),
    ((275, 277, 279, 300), _ALL, 0), ((296, 236, 292, 256), _ALL, 1),
    ((285, 307, 323, 235), _ALL, 0), ((272, 286, 290, 268), _ALL, 0),
    ((264, 299, 258, 301), _ALL, 0), ((222, 274, 322, 278), _ALL, 0),
    ((281, 232, 297, 273), _ALL, 0), ((309, 318, 294, 282), _ALL, 0),
    ((317, 227, 223, 225), _ALL, 0), ((233, 257, 259, 255), _ALL, 0),
    ((253, 270, 251, 243), _ALL, 0), ((241, 269, 271, 230), _ALL, 1),
    ((246, 240, 248, 247), _ALL, 0), ((242, 244, 226, 315), _ALL, 0),
    ((220, 216, 217, 221), _ALL, 0), ((312, 313, 314, 219), _ALL, 0),
)


def _signed_sum(terms):
    sign, total = terms[0]
    for s, value in terms[1:]:
        if s == sign:
            total = total + value
        elif sign > 0:
            total = total - value
        else:
            sign, total = 1, value - total
    return sign, total


@jax.jit
def pallas_standalone__glu_gated_bilinear__prompt_kernel(
    x: jax.Array,
    w_gate: jax.Array,
    w_up: jax.Array,
    w_down: jax.Array,
):
    batch, seq, d_model = x.shape
    tokens, d_ff = batch * seq, w_gate.shape[1]
    assert (d_model, d_ff) == (5 * T, 13 * T + HALF) and tokens % (2 * ROWS) == 0
    n_tiles = tokens // (2 * ROWS)
    f32, mxu_dtype = jnp.float32, jnp.bfloat16
    products = _all_products()
    covered = sorted((p, b) for ids, blocks, _ in _STEPS for p in ids for b in blocks)
    assert covered == [(p, b) for p in range(len(products)) for b in _ALL]

    def kernel(x_hbm, wg_hbm, wu_hbm, wd_hbm, out_hbm,
               x_buf, wg_buf, wu_buf, wd_buf, early_buf, out_buf, in_sems, out_sem):
        hbm = dict(x=x_hbm, g=wg_hbm, u=wu_hbm, d=wd_hbm, e=wg_hbm)
        vmem = dict(x=x_buf, g=wg_buf, u=wu_buf, d=wd_buf, e=early_buf)
        first_row = dict(x=0, g=0, u=0, d=0, e=10 * T)

        def copy(tile, i):
            name, (r0, r1), (c0, c1), _ = _COPIES[i]
            rows = (r1 * T if name == "x" else min(r1 * T, d_ff)) - r0 * T
            cols = pl.ds(c0 * T, (c1 - c0) * T)
            src_row = tile * 2 * ROWS + r0 * T if name == "x" else r0 * T
            return pltpu.make_async_copy(
                hbm[name].at[pl.ds(src_row, rows), cols],
                vmem[name].at[tile, pl.ds(r0 * T - first_row[name], rows), cols],
                in_sems.at[tile * len(_COPIES) + i])

        for tile in range(n_tiles):
            for i in range(len(_COPIES)):
                copy(tile, i).start()

        def token_tile(tile, carry):
            in_flight = list(range(len(_COPIES)))
            buf = {name: ref.at[tile] for name, ref in vmem.items()}

            def wait(i):
                copy(tile, i).wait()
                in_flight.remove(i)

            def load(name, row, rows, col_tile):
                for i in list(in_flight):
                    other, (r0, r1), (c0, c1), _ = _COPIES[i]
                    if other == name and r0 * T <= row < r1 * T and c0 <= col_tile < c1:
                        wait(i)
                row -= first_row[name]
                return buf[name][row:row + rows, col_tile * T:(col_tile + 1) * T]

            def weight_tile(stage, k, n):
                if stage == 1:
                    kind, f = n
                    if kind == "m":
                        return jnp.concatenate([load(w, f * T, HALF, k) for w in "gu"], axis=0)
                    return load(kind, f * T, T, k)
                if k in ("T", "B"):
                    halves = (2, 1) if k == "T" else (0, 2)
                    return jnp.concatenate(
                        [load("d", 12 * T + j * HALF, HALF, n) for j in halves], axis=0)
                return load("d", (12 if k == "D" else k) * T, T, n)

            def operand(terms, get):
                terms = sorted(terms, key=lambda term: -term[0])
                return _signed_sum([(s, get(*key).astype(f32)) for s, *key in terms])[1].astype(mxu_dtype)

            hidden, operands = {}, {}
            low_lanes = lax.broadcasted_iota(jnp.int32, (BLOCK, T), 1) < HALF

            def activation(stage, b, h, k):
                if stage == 1:
                    return load("x", h * ROWS + b * BLOCK, BLOCK, k)
                if (h, k, b) not in hidden:
                    top, bottom = hidden[0, 12, b], hidden[1, 12, b]
                    if k == "T":
                        hidden[h, k, b] = jnp.where(low_lanes, hidden[0, 13, b], top + bottom)
                    elif k == "B":
                        hidden[h, k, b] = jnp.where(low_lanes, top + bottom, hidden[1, 13, b])
                    else:
                        hidden[h, k, b] = jnp.where(low_lanes, top, -bottom)
                return hidden[h, k, b]

            def left_operand(stage, lhs, b):
                if stage == 1 and len(lhs) == 1:
                    return activation(stage, b, *lhs[0][1:]).astype(mxu_dtype)
                if (stage, lhs, b) not in operands:
                    operands[stage, lhs, b] = operand(lhs, lambda h, k: activation(stage, b, h, k))
                return operands[stage, lhs, b]

            def right_operand(stage, rhs):
                if len(rhs) == 1:
                    return weight_tile(stage, *rhs[0][1:]).astype(mxu_dtype)
                return operand(rhs, lambda k, n: weight_tile(stage, k, n))

            missing, partial = {}, {}
            for stage, _, _, dst in products:
                for _, h, n in dst:
                    for b in _ALL:
                        missing[stage, h, n, b] = missing.get((stage, h, n, b), 0) + 1

            def value(key):
                sign, total = _signed_sum(partial[key])
                return total if sign > 0 else -total

            for step, (ids, blocks, defer) in enumerate(_STEPS):
                for i in list(in_flight):
                    if _COPIES[i][3] <= step:
                        wait(i)
                whole = len(ids) * len(blocks) > 4
                results = {}
                for p in ids:
                    stage, lhs, rhs, _ = products[p]
                    if stage == 1 and not whole and rhs[0][2][1] >= 10:
                        rhs = ((1, rhs[0][1], ("e", rhs[0][2][1])),)
                    for piece in [blocks] if whole else [(b,) for b in blocks]:
                        a = jnp.concatenate([left_operand(stage, lhs, b) for b in piece], axis=0)
                        contract = ((1,), (1 if stage == 1 else 0,))
                        r = lax.dot_general(a, right_operand(stage, rhs), (contract, ((), ())),
                                            preferred_element_type=f32)
                        for j, b in enumerate(piece):
                            results[p, b] = r[j * BLOCK:(j + 1) * BLOCK]

                for b in blocks:
                    arrived = {}
                    for p in ids:
                        stage, _, _, dst = products[p]
                        for s, h, n in dst:
                            arrived.setdefault((stage, h, n, b), []).append((s, results[p, b]))
                    for key, terms in arrived.items():
                        missing[key] -= len(terms)
                        earlier = partial.get(key, [])
                        keep_aside = defer and len(terms) == 1 and len(earlier) < 3
                        partial[key] = terms + earlier if keep_aside else [_signed_sum(terms + earlier)]
                    done = [key for key in arrived if not missing[key]]
                    size = BLOCK // 4 if step == len(_STEPS) - 1 else BLOCK
                    totals = {key: value(key) for key in done if key[0] == 2}
                    for r0 in range(0, BLOCK, size):
                        for (_, h, n, _), total in totals.items():
                            rows = pl.ds(tile * 2 * ROWS + h * ROWS + b * BLOCK + r0, size)
                            cols = pl.ds(n * T, T)
                            out_buf[n, rows, :] = total[r0:r0 + size].astype(out_buf.dtype)
                            pltpu.make_async_copy(
                                out_buf.at[n, rows], out_hbm.at[rows, cols], out_sem).start()
                    for key in done:
                        stage, h, n, _ = key
                        if stage == 2:
                            continue
                        if n[0] == "m":
                            both = value(key)
                            hidden[h, n[1], b] = both * pltpu.roll(both, HALF, 1)
                        elif (h, n[1], b) not in hidden:
                            other = (1, h, ("u" if n[0] == "g" else "g", n[1]), b)
                            if not missing[other]:
                                hidden[h, n[1], b] = value(key) * value(other)
            assert not in_flight and not any(missing.values())
            return carry

        lax.fori_loop(0, n_tiles, token_tile, 0)
        pltpu.make_async_copy(out_hbm, out_hbm, out_sem).wait()

    any_hbm = pl.BlockSpec(memory_space=pltpu.HBM)
    out = pl.pallas_call(
        kernel,
        in_specs=[any_hbm] * 4,
        out_specs=any_hbm,
        out_shape=jax.ShapeDtypeStruct((tokens, d_model), x.dtype),
        scratch_shapes=[
            pltpu.VMEM((n_tiles, 2 * ROWS, d_model), x.dtype),
            pltpu.VMEM((n_tiles, d_ff, d_model), w_gate.dtype),
            pltpu.VMEM((n_tiles, d_ff, d_model), w_up.dtype),
            pltpu.VMEM((n_tiles, d_ff, d_model), w_down.dtype),
            pltpu.VMEM((n_tiles, 2 * T, 2 * T), w_gate.dtype),
            pltpu.VMEM((d_model // T, tokens, T), x.dtype),
            pltpu.SemaphoreType.DMA((n_tiles * len(_COPIES),)),
            pltpu.SemaphoreType.DMA(()),
        ],
        compiler_params=pltpu.CompilerParams(
            vmem_limit_bytes=100 * 1024 * 1024,
            flags={"XLA_TPU_RESCHEDULE_DMA_DONES": True},
            disable_semaphore_checks=True,
        ),
    )(x.reshape(tokens, d_model), w_gate.T, w_up.T, w_down)
    return out.reshape(batch, seq, d_model)
```
